```python
import jax
import jax.numpy as jnp

def _softmax(x, axis=-1):
    return jax.nn.softmax(x, axis=axis)
def _gelu(x):
    return jax.nn.gelu(x, approximate=True)
def _silu(x):
    return jax.nn.silu(x)
def _sigmoid(x):
    return jax.nn.sigmoid(x)
def _layernorm(x, axis=-1, eps=1e-5):
    m = jnp.mean(x, axis=axis, keepdims=True)
    v = jnp.var(x, axis=axis, keepdims=True)
    return (x - m) / jnp.sqrt(v + eps)
def _scatter_add(tgt, idx, src, axis=0):
    return tgt.at[idx].add(src)
def _segment_sum(src, seg, n):
    return jax.ops.segment_sum(src, seg, n)
class _Rng:
    def __init__(self, key):
        self._k = key
    def _next(self):
        self._k, sub = jax.random.split(self._k)
        return sub
    def normal(self, shape):
        return jax.random.normal(self._next(), shape, dtype=jnp.bfloat16)
    def randint(self, lo, hi, shape):
        return jax.random.randint(self._next(), shape, lo, hi, dtype=jnp.int32)
    def uniform(self, shape, lo=0.0, hi=1.0):
        return jax.random.uniform(self._next(), shape, jnp.bfloat16, lo, hi)
    def permutation(self, n):
        return jax.random.permutation(self._next(), n)


kernel_name = 'standalone__standard_2d_1d_3d_conv__vision'

def setup_inputs():
    _rng = _Rng(jax.random.key(int.from_bytes(__import__("os").urandom(4), "little")))
    _w = (lambda a: (lambda t: t.astype(jnp.bfloat16) if jnp.issubdtype(t.dtype, jnp.floating) else t)(jnp.asarray(a)))
    H = W = 384
    C = 384
    K = 1
    return {
        "x": _w((lambda *s: _rng.normal(s) * 0.05)(1, H, W, C)),
        "w": _w((lambda *s: _rng.normal(s) * 0.05)(K, K, C, C)),
        "b": _w((lambda *s: _rng.normal(s) * 0.05)(C)),
    }

def reference(x, w, b):
    B, H, W, Cin = x.shape
    K = w.shape[0]
    pl = (K - 1) // 2
    pr = K // 2
    xp = jnp.pad(x, ((0, 0), (pl, pr), (pl, pr), (0, 0)))
    out = sum(
        jnp.einsum('bhwc,cd->bhwd', xp[:, i:i+H, j:j+W, :], w[i, j])
        for i in range(K) for j in range(K)
    )
    return out + b[None, None, None, :]
```

```python
import jax
import jax.numpy as jnp
import jax.experimental.pallas as pl
import jax.experimental.pallas.tpu as pltpu


def _conv1x1_kernel(x_ref, w_ref, b_ref, o_ref):
    acc = jnp.dot(x_ref[...], w_ref[...], preferred_element_type=jnp.float32)
    o_ref[...] = (acc + b_ref[...].astype(jnp.float32)).astype(o_ref.dtype)


@jax.jit
def pallas_standalone__standard_2d_1d_3d_conv__vision_kernel(
    x: jax.Array,
    w: jax.Array,
    b: jax.Array,
):
    B, H, W, Cin = x.shape
    K, _, _, Cout = w.shape
    assert K == 1
    M = B * H * W
    bm = 4096
    out = pl.pallas_call(
        _conv1x1_kernel,
        grid=(M // bm,),
        in_specs=[
            pl.BlockSpec((bm, Cin), lambda i: (i, 0)),
            pl.BlockSpec((Cin, Cout), lambda i: (0, 0)),
            pl.BlockSpec((1, Cout), lambda i: (0, 0)),
        ],
        out_specs=pl.BlockSpec((bm, Cout), lambda i: (i, 0)),
        out_shape=jax.ShapeDtypeStruct((M, Cout), x.dtype),
        compiler_params=pltpu.CompilerParams(
            dimension_semantics=("arbitrary",),
            vmem_limit_bytes=100 * 1024 * 1024,
        ),
    )(x.reshape(M, Cin), w.reshape(Cin, Cout), b.reshape(1, Cout))
    return out.reshape(B, H, W, Cout)
```

```python
import functools

import jax
import jax.numpy as jnp
import jax.experimental.pallas as pl
import jax.experimental.pallas.tpu as pltpu

_STREAMS = 6
_WRITE_ROWS = 48
_TILE_ROWS = 384
_TILES_PER_READ = 4
_SWITCH_TILE = 35
_FIRST_WRITES = 48
_WRITES_PER_TILE = 16
_TAIL_ROWS = 96


def _conv1x1_kernel(x_hbm, w_hbm, b_hbm, o_hbm, buf, w_vmem, b_vmem, bias_ref,
                    read_sems, param_sems, write_sem):
    streams, rows, cin = buf.shape
    cout = w_vmem.shape[1]
    n_tiles = rows // _TILE_ROWS
    n_reads = n_tiles // _TILES_PER_READ
    n_writes = rows // _WRITE_ROWS
    read_rows = _TILE_ROWS * _TILES_PER_READ

    def read(start, size, sem_index):
        rows_slice = pl.ds(start, size)
        return pltpu.make_async_copy(
            x_hbm.at[:, rows_slice], buf.at[:, rows_slice], read_sems.at[sem_index])

    def read_group(i):
        return read(pl.multiple_of(i * read_rows, read_rows), read_rows, i)

    def read_last_group():
        return read((n_reads - 1) * read_rows, read_rows - _TAIL_ROWS, n_reads - 1)

    def read_tail():
        return read(rows - _TAIL_ROWS, _TAIL_ROWS, n_reads)

    def start_write(j, _):
        rows_slice = pl.ds(pl.multiple_of(j * _WRITE_ROWS, _WRITE_ROWS), _WRITE_ROWS)
        pltpu.make_async_copy(
            buf.at[:, rows_slice], o_hbm.at[:, rows_slice], write_sem).start()

    w_copy = pltpu.make_async_copy(w_hbm, w_vmem, param_sems.at[0])
    b_copy = pltpu.make_async_copy(b_hbm, b_vmem, param_sems.at[1])
    w_copy.start()
    b_copy.start()
    jax.lax.fori_loop(0, n_reads - 1, lambda i, _: read_group(i).start(), None)
    w_copy.wait()
    b_copy.wait()
    read_last_group().start()
    bias_ref[...] = jnp.broadcast_to(
        b_vmem[...].astype(jnp.float32).reshape(1, cout), bias_ref.shape)

    def tile_step(t, _):
        @pl.when(jnp.logical_and(t < _SWITCH_TILE, t % _TILES_PER_READ == 0))
        def _():
            read_group(t // _TILES_PER_READ).wait()

        @pl.when(t == 1)
        def _():
            read_tail().start()

        @pl.when(t == _SWITCH_TILE)
        def _():
            for i in range(pl.cdiv(_SWITCH_TILE, _TILES_PER_READ), n_reads - 1):
                read_group(i).wait()
            read_last_group().wait()
            jax.lax.fori_loop(0, _FIRST_WRITES, start_write, None)
            read_tail().wait()

        rows_slice = pl.ds(pl.multiple_of(t * _TILE_ROWS, _TILE_ROWS), _TILE_ROWS)
        x_tile = buf[:, rows_slice, :].reshape(streams * _TILE_ROWS, cin)
        acc = jnp.dot(x_tile, w_vmem[...], preferred_element_type=jnp.float32)
        acc = acc + bias_ref[0:1, :]
        buf[:, rows_slice, :] = acc.astype(buf.dtype).reshape(streams, _TILE_ROWS, cout)

        @pl.when(t >= _SWITCH_TILE)
        def _():
            first = _FIRST_WRITES + (t - _SWITCH_TILE) * _WRITES_PER_TILE
            jax.lax.fori_loop(first, first + _WRITES_PER_TILE, start_write, None)

    assert _FIRST_WRITES * _WRITE_ROWS <= _SWITCH_TILE * _TILE_ROWS
    for t in range(_SWITCH_TILE, n_tiles):
        queued = _FIRST_WRITES + (t - _SWITCH_TILE + 1) * _WRITES_PER_TILE
        assert queued * _WRITE_ROWS <= (t + 1) * _TILE_ROWS
    assert queued == n_writes
    assert pl.cdiv(_SWITCH_TILE, _TILES_PER_READ) <= n_reads - 1

    jax.lax.fori_loop(0, n_tiles, tile_step, None)
    pltpu.make_async_copy(buf, o_hbm, write_sem).wait()


@jax.jit
def pallas_standalone__standard_2d_1d_3d_conv__vision_kernel(
    x: jax.Array,
    w: jax.Array,
    b: jax.Array,
):
    B, H, W, Cin = x.shape
    K, _, _, Cout = w.shape
    assert K == 1 and Cin == Cout
    rows = B * H * W // _STREAMS
    n_reads = rows // (_TILE_ROWS * _TILES_PER_READ)
    assert n_reads * _TILE_ROWS * _TILES_PER_READ * _STREAMS == B * H * W
    hbm = pl.BlockSpec(memory_space=pltpu.HBM)
    out = pl.pallas_call(
        _conv1x1_kernel,
        in_specs=[hbm, hbm, hbm],
        out_specs=hbm,
        out_shape=jax.ShapeDtypeStruct((_STREAMS, rows, Cout), x.dtype),
        scratch_shapes=[
            pltpu.VMEM((_STREAMS, rows, Cin), x.dtype),
            pltpu.VMEM((Cin, Cout), w.dtype),
            pltpu.VMEM((Cout,), b.dtype),
            pltpu.VMEM((8, Cout), jnp.float32),
            pltpu.SemaphoreType.DMA((n_reads + 1,)),
            pltpu.SemaphoreType.DMA((2,)),
            pltpu.SemaphoreType.DMA(()),
        ],
        compiler_params=pltpu.CompilerParams(vmem_limit_bytes=127 * 1024 * 1024),
    )(x.reshape(_STREAMS, rows, Cin), w.reshape(Cin, Cout), b)
    return out.reshape(B, H, W, Cout)
```

```python
import jax
import jax.numpy as jnp
from jax import lax
import jax.experimental.pallas as pl
import jax.experimental.pallas.tpu as pltpu

_LANES = 128
_SUBLANES = 8
_COL_TILES = 3
_REGION_ROWS = 4096
_STREAMS = 6
_WRITE_ROWS = 64
_TILE_ROWS = 2048

_READ_GROUPS = (0, 6, 15, 27, 42, 60)
_TAIL_ROWS = 32
_FIRST_WRITES = 48
_WRITES_PER_TILE = 33


def _divmod_pow2(i, n):
    assert n & (n - 1) == 0
    return lax.shift_right_logical(i, n.bit_length() - 1), i & (n - 1)


def _tiles_to_rows(x):
    rows = x.shape[0] // _COL_TILES
    v = pltpu.bitcast(x, jnp.uint32).reshape(-1, _COL_TILES, _SUBLANES, _LANES)
    v0, v1, v2 = v[:, 0], v[:, 1], v[:, 2]
    low = lax.broadcasted_iota(jnp.int32, v0.shape, 1) < _SUBLANES // 2
    cols = (
        jnp.where(low, v0, v1),
        pltpu.roll(jnp.where(low, v2, v0), _SUBLANES // 2, 1),
        jnp.where(low, v1, v2),
    )
    cols = [c.reshape(rows // 2, _LANES) for c in cols]
    return pltpu.bitcast(jnp.concatenate(cols, axis=1), x.dtype)


def _rows_to_tiles(y):
    cols = [
        y[:, j * _LANES:(j + 1) * _LANES].reshape(-1, _SUBLANES, _LANES)
        for j in range(_COL_TILES)
    ]
    return jnp.stack(cols, axis=1).reshape(-1, _LANES)


def _conv1x1_kernel(x_hbm, w_hbm, b_hbm, o_hbm, buf, w_vmem, b_vmem, bias_ref, sems):
    regions = buf.shape[0]
    n_groups = len(_READ_GROUPS)
    n_tiles = regions * _REGION_ROWS // (_COL_TILES * _TILE_ROWS)
    writes_per_block = _REGION_ROWS // _WRITE_ROWS
    n_writes = regions // _STREAMS * writes_per_block
    group_tile = [r * _REGION_ROWS // (_COL_TILES * _TILE_ROWS) for r in _READ_GROUPS]
    switch_tile = group_tile[-1]

    def read_group(k):
        if k < n_groups - 1:
            idx = (pl.ds(_READ_GROUPS[k], _READ_GROUPS[k + 1] - _READ_GROUPS[k]),)
        else:
            head_rows = _REGION_ROWS - _TAIL_ROWS
            idx = (
                pl.ds(_READ_GROUPS[-1], regions - _READ_GROUPS[-1]),
                pl.ds(0, head_rows) if k < n_groups else pl.ds(head_rows, _TAIL_ROWS),
            )
        return pltpu.make_async_copy(x_hbm.at[idx], buf.at[idx], sems.at[k % 2])

    write_sem = sems.at[(n_groups - 1) % 2]

    def start_write(j, _):
        block, piece = _divmod_pow2(j, writes_per_block)
        idx = (
            pl.ds(block * _STREAMS, _STREAMS),
            pl.ds(pl.multiple_of(piece * _WRITE_ROWS, _WRITE_ROWS), _WRITE_ROWS),
        )
        pltpu.make_async_copy(buf.at[idx], o_hbm.at[idx], write_sem).start()

    w_copy = pltpu.make_async_copy(w_hbm, w_vmem, sems.at[0])
    b_copy = pltpu.make_async_copy(b_hbm, b_vmem, sems.at[0])
    w_copy.start()
    b_copy.start()
    read_group(0).start()

    def enter_group(k):
        if k == 0:
            read_group(1).start()
            w_copy.wait()
            b_copy.wait()
        read_group(k).wait()
        if k == 0:
            bias = b_vmem[...].astype(jnp.float32).reshape(1, -1)
            bias_ref[...] = jnp.broadcast_to(bias, bias_ref.shape)
        if k + 2 <= n_groups:
            read_group(k + 2).start()
        if k == n_groups - 1:
            lax.fori_loop(0, _FIRST_WRITES, start_write, None)
            read_group(n_groups).wait()

    def tile_step(t, _):
        for k in range(n_groups):
            pl.when(t == group_tile[k])(lambda k=k: enter_group(k))

        def third(k):
            region, part = _divmod_pow2(_COL_TILES * t + k, _REGION_ROWS // _TILE_ROWS)
            return region, pl.ds(pl.multiple_of(part * _TILE_ROWS, _TILE_ROWS), _TILE_ROWS)

        x = _tiles_to_rows(jnp.concatenate([buf[third(k)] for k in range(_COL_TILES)]))
        y = jnp.dot(x, w_vmem[...], preferred_element_type=jnp.float32)
        y = _rows_to_tiles(y + bias_ref[0:1, :])
        for k in range(_COL_TILES):
            buf[third(k)] = y[k * _TILE_ROWS:(k + 1) * _TILE_ROWS].astype(buf.dtype)

        @pl.when(t >= switch_tile)
        def _():
            first = _FIRST_WRITES + (t - switch_tile) * _WRITES_PER_TILE
            lax.fori_loop(first, first + _WRITES_PER_TILE, start_write, None)

    def writes_ready(tiles_done):
        blocks = tiles_done * _COL_TILES * _TILE_ROWS // (_STREAMS * _REGION_ROWS)
        return blocks * writes_per_block

    for t in range(switch_tile, n_tiles + 1):
        assert _FIRST_WRITES + (t - switch_tile) * _WRITES_PER_TILE <= writes_ready(t)
    for k in range(n_groups):
        assert group_tile[k] * _COL_TILES * _TILE_ROWS == _READ_GROUPS[k] * _REGION_ROWS

    lax.fori_loop(0, n_tiles, tile_step, None)
    queued = _FIRST_WRITES + (n_tiles - switch_tile) * _WRITES_PER_TILE
    lax.fori_loop(queued, n_writes, start_write, None)
    pltpu.make_async_copy(buf, o_hbm, write_sem).wait()


@jax.jit
def pallas_standalone__standard_2d_1d_3d_conv__vision_kernel(
    x: jax.Array,
    w: jax.Array,
    b: jax.Array,
):
    B, H, W, C = x.shape
    assert w.shape == (1, 1, C, C) and C == _COL_TILES * _LANES
    row_groups = B * H * W // _SUBLANES
    regions = B * H * W * _COL_TILES // _REGION_ROWS
    assert regions * _REGION_ROWS == B * H * W * _COL_TILES and regions % _STREAMS == 0

    tiled_shape = (regions, _REGION_ROWS, _LANES)
    x_tiled = x.reshape(row_groups, _SUBLANES, _COL_TILES, _LANES)
    x_tiled = x_tiled.transpose(0, 2, 1, 3).reshape(tiled_shape)
    hbm = pl.BlockSpec(memory_space=pltpu.HBM)
    out = pl.pallas_call(
        _conv1x1_kernel,
        in_specs=[hbm, hbm, hbm],
        out_specs=hbm,
        out_shape=jax.ShapeDtypeStruct(tiled_shape, x.dtype),
        scratch_shapes=[
            pltpu.VMEM(tiled_shape, x.dtype),
            pltpu.VMEM((C, C), w.dtype),
            pltpu.VMEM((C,), b.dtype),
            pltpu.VMEM((_SUBLANES, C), jnp.float32),
            pltpu.SemaphoreType.DMA((2,)),
        ],
        compiler_params=pltpu.CompilerParams(vmem_limit_bytes=120 * 1024 * 1024),
    )(x_tiled, w.reshape(C, C), b)
    out = out.reshape(row_groups, _COL_TILES, _SUBLANES, _LANES)
    return out.transpose(0, 2, 1, 3).reshape(B, H, W, C)
```
